```python
import jax
import jax.numpy as jnp

def _softmax(x, axis=-1):
    return jax.nn.softmax(x, axis=axis)
def _gelu(x):
    return jax.nn.gelu(x, approximate=True)
def _silu(x):
    return jax.nn.silu(x)
def _sigmoid(x):
    return jax.nn.sigmoid(x)
def _layernorm(x, axis=-1, eps=1e-5):
    m = jnp.mean(x, axis=axis, keepdims=True)
    v = jnp.var(x, axis=axis, keepdims=True)
    return (x - m) / jnp.sqrt(v + eps)
def _scatter_add(tgt, idx, src, axis=0):
    return tgt.at[idx].add(src)
def _segment_sum(src, seg, n):
    return jax.ops.segment_sum(src, seg, n)
class _Rng:
    def __init__(self, key):
        self._k = key
    def _next(self):
        self._k, sub = jax.random.split(self._k)
        return sub
    def normal(self, shape):
        return jax.random.normal(self._next(), shape, dtype=jnp.bfloat16)
    def randint(self, lo, hi, shape):
        return jax.random.randint(self._next(), shape, lo, hi, dtype=jnp.int32)
    def uniform(self, shape, lo=0.0, hi=1.0):
        return jax.random.uniform(self._next(), shape, jnp.bfloat16, lo, hi)
    def permutation(self, n):
        return jax.random.permutation(self._next(), n)


kernel_name = 'parallel_sum__sliding_block_cached__mixer_s_mlp__decode'

def setup_inputs():
    _rng = _Rng(jax.random.key(int.from_bytes(__import__("os").urandom(4), "little")))
    _w = (lambda a: (lambda t: t.astype(jnp.bfloat16) if jnp.issubdtype(t.dtype, jnp.floating) else t)(jnp.asarray(a)))
    def _A_setup():
        B, Sq, D = 4, 1, 512
        Hq, Hkv, Sk, Dh = 32, 32, 8192, 128
        assert Hq % Hkv == 0, (Hq, Hkv)
        return {
            "x": _w((lambda *s: _rng.normal(s) * 0.05)(B, Sq, D)),
            "k_cache": _w((lambda *s: _rng.normal(s) * 0.05)(B, Hkv, Sk, Dh)),
            "v_cache": _w((lambda *s: _rng.normal(s) * 0.05)(B, Hkv, Sk, Dh)),
            "wq": _w((lambda *s: _rng.normal(s) * 0.05)(D, Hq * Dh) * (D ** -0.5)),
            "wo": _w((lambda *s: _rng.normal(s) * 0.05)(Hq * Dh, D) * ((Hq * Dh) ** -0.5)),
        }
    _A_in = _A_setup()

    def _B_setup():
        B, S, D, F = 4, 1, 512, 1376
        return {
            "x":  _w((lambda *s: _rng.normal(s) * 0.05)(B, S, D)),
            "w1": _w((lambda *s: _rng.normal(s) * 0.05)(D, D) * (D ** -0.5)),
            "w2": _w((lambda *s: _rng.normal(s) * 0.05)(D, D) * (D ** -0.5)),
            "w3": _w((lambda *s: _rng.normal(s) * 0.05)(D, F) * (D ** -0.5)),
            "w4": _w((lambda *s: _rng.normal(s) * 0.05)(F, D) * (F ** -0.5)),
        }
    _B_in = _B_setup()

    return {
        "A_x": _A_in["x"],
        "A_k_cache": _A_in["k_cache"],
        "A_v_cache": _A_in["v_cache"],
        "A_wq": _A_in["wq"],
        "A_wo": _A_in["wo"],
        "B_x": _B_in["x"],
        "B_w1": _B_in["w1"],
        "B_w2": _B_in["w2"],
        "B_w3": _B_in["w3"],
        "B_w4": _B_in["w4"],
    }

def reference(A_x, A_k_cache, A_v_cache, A_wq, A_wo, B_x, B_w1, B_w2, B_w3, B_w4):
    def _A_ref(x, k_cache, v_cache, wq, wo):
        B, Sq, D = x.shape
        Hq, Dh = 32, 128
        Hkv, Sk = k_cache.shape[1], k_cache.shape[2]
        W = min(4096, max(256, Sk // 4))
        rep = Hq // Hkv
        q = (lambda x, *d: x.transpose(*d))((x @ wq).reshape(B, Sq, Hq, Dh), 0, 2, 1, 3)
        k = jnp.repeat(k_cache[:, :, Sk - W:, :], rep, axis=1)
        v = jnp.repeat(v_cache[:, :, Sk - W:, :], rep, axis=1)
        scores = jnp.einsum("bhqd,bhkd->bhqk", q, k) * (Dh ** -0.5)
        p = _softmax(scores, axis=-1)
        o = jnp.einsum("bhqk,bhkd->bhqd", p, v)
        return (lambda x, *d: x.transpose(*d))(o, 0, 2, 1, 3).reshape(B, Sq, Hq * Dh) @ wo

    def _B_ref(x, w1, w2, w3, w4):
        B, S, D = x.shape
        h = _gelu(_layernorm(x, axis=-1) @ w1)
        c = D // 4
        g0 = jnp.pad(h[:, :, 0*c:1*c], ((0, 0), (1, 0), (0, 0)))[:, :S, :]
        g1 = jnp.pad(h[:, :, 1*c:2*c], ((0, 0), (0, 1), (0, 0)))[:, 1:, :]
        g2 = jnp.pad(h[:, :, 2*c:3*c], ((0, 0), (2, 0), (0, 0)))[:, :S, :]
        g3 = jnp.pad(h[:, :, 3*c:   ], ((0, 0), (0, 2), (0, 0)))[:, 2:, :]
        hs = jnp.concatenate([g0, g1, g2, g3], axis=-1) @ w2
        x1 = x + hs
        h2 = _gelu(_layernorm(x1, axis=-1) @ w3) @ w4
        return x1 + h2

    x = A_x
    xn = _layernorm(x, axis=-1)
    return x + _A_ref(xn, A_k_cache, A_v_cache, A_wq, A_wo) + _B_ref(xn, B_w1, B_w2, B_w3, B_w4)
```

```python
import functools

import jax
import jax.numpy as jnp
import jax.experimental.pallas as pl
import jax.experimental.pallas.tpu as pltpu

_EPS = 1e-5
_NBUF = 8
_WO_CHUNKS = 8


def _layernorm(x):
    m = jnp.mean(x, axis=-1, keepdims=True)
    xc = x - m
    v = jnp.mean(xc * xc, axis=-1, keepdims=True)
    return xc / jnp.sqrt(v + _EPS)


def _make_kernel(B, H, SK, DH, W, D, F):
    NP = B * H
    HPC = H // _WO_CHUNKS
    scale = DH ** -0.5

    def kernel(x_hbm, k_hbm, v_hbm, wq_hbm, wo_hbm, w3_hbm, w4_hbm, out_hbm,
               x_buf, kbuf, vbuf, wq_buf, wo_buf, w3_buf, w4_buf,
               q_scr, o_scr, out_buf,
               sem_k, sem_v, sem_w, sem_wo):
        x_cp = pltpu.make_async_copy(x_hbm, x_buf, sem_w.at[0])
        w3_cp = pltpu.make_async_copy(w3_hbm, w3_buf, sem_w.at[1])
        w4_cp = pltpu.make_async_copy(w4_hbm, w4_buf, sem_w.at[2])
        wq_cp = pltpu.make_async_copy(wq_hbm, wq_buf, sem_w.at[3])
        out_cp = pltpu.make_async_copy(out_buf, out_hbm, sem_w.at[4])

        def k_cp(b, h, slot):
            return pltpu.make_async_copy(
                k_hbm.at[b, h, pl.ds(SK - W, W), :], kbuf.at[slot], sem_k.at[slot])

        def v_cp(b, h, slot):
            return pltpu.make_async_copy(
                v_hbm.at[b, h, pl.ds(SK - W, W), :], vbuf.at[slot], sem_v.at[slot])

        def wo_cp(c):
            rows = HPC * DH
            return pltpu.make_async_copy(
                wo_hbm.at[pl.ds(c * rows, rows), :], wo_buf.at[pl.ds(c * rows, rows), :],
                sem_wo.at[c])

        x_cp.start()
        w3_cp.start()
        w4_cp.start()
        wq_cp.start()
        for p in range(_NBUF):
            k_cp(p % B, p // B, p).start()
            v_cp(p % B, p // B, p).start()

        x_cp.wait()
        x4 = x_buf[...].astype(jnp.float32)
        x8 = jnp.concatenate([x4, x4], axis=0)
        xn = _layernorm(x8)
        xn2 = _layernorm(xn)
        w3_cp.wait()
        hmid = jax.lax.dot_general(xn2.astype(jnp.bfloat16), w3_buf[...], (((1,), (1,)), ((), ())),
                                   preferred_element_type=jnp.float32)
        hmid = jax.nn.gelu(hmid, approximate=True)
        w4_cp.wait()
        mlp = jnp.dot(hmid.astype(jnp.bfloat16), w4_buf[...], preferred_element_type=jnp.float32)
        base = x8 + xn + mlp

        wq_cp.wait()
        q_all = jnp.dot(xn.astype(jnp.bfloat16), wq_buf[...], preferred_element_type=jnp.float32)
        for h in range(H):
            q_scr[h] = q_all[:, h * DH:(h + 1) * DH]

        row = jax.lax.broadcasted_iota(jnp.int32, (8, DH), 0)

        def head_body(h, carry):
            q = q_scr[h].astype(jnp.bfloat16)
            o_h = jnp.zeros((8, DH), jnp.float32)
            for b in range(B):
                slot = (h * B + b) % _NBUF
                k_cp(b, h, slot).wait()
                s = jax.lax.dot_general(q, kbuf[slot], (((1,), (1,)), ((), ())),
                                        preferred_element_type=jnp.float32)
                m = jnp.max(s, axis=-1, keepdims=True)
                p = jnp.exp((s - m) * scale)
                l = jnp.sum(p, axis=-1, keepdims=True)
                v_cp(b, h, slot).wait()
                o = jnp.dot(p.astype(jnp.bfloat16), vbuf[slot],
                            preferred_element_type=jnp.float32)
                o_h = jnp.where((row % B) == b, o / l, o_h)
                hn = h + _NBUF // B

                @pl.when(hn < H)
                def _():
                    k_cp(b, hn, slot).start()
                    v_cp(b, hn, slot).start()

                if b == B - 1:
                    @pl.when(hn == H)
                    def _():
                        for c in range(_WO_CHUNKS):
                            wo_cp(c).start()
            o_scr[h] = o_h
            return carry

        jax.lax.fori_loop(0, H, head_body, 0)

        acc = base
        for c in range(_WO_CHUNKS):
            wo_cp(c).wait()
            for hh in range(HPC):
                h = c * HPC + hh
                acc = acc + jnp.dot(o_scr[h].astype(jnp.bfloat16), wo_buf[h * DH:(h + 1) * DH, :],
                                    preferred_element_type=jnp.float32)
        out_buf[...] = acc[0:B, :].astype(out_buf.dtype)
        out_cp.start()
        out_cp.wait()

    return kernel


@jax.jit
def pallas_parallel_sum__sliding_block_cached__mixer_s_mlp__decode_kernel(
    A_x: jax.Array,
    A_k_cache: jax.Array,
    A_v_cache: jax.Array,
    A_wq: jax.Array,
    A_wo: jax.Array,
    B_x: jax.Array,
    B_w1: jax.Array,
    B_w2: jax.Array,
    B_w3: jax.Array,
    B_w4: jax.Array,
):
    B, SQ, D = A_x.shape
    _, H, SK, DH = A_k_cache.shape
    F = B_w3.shape[1]
    W = min(4096, max(256, SK // 4))
    assert SQ == 1 and B == 4 and H % _WO_CHUNKS == 0 and _NBUF % B == 0
    dt = A_x.dtype

    any_spec = pl.BlockSpec(memory_space=pl.ANY)
    out = pl.pallas_call(
        _make_kernel(B, H, SK, DH, W, D, F),
        out_shape=jax.ShapeDtypeStruct((B, D), dt),
        in_specs=[any_spec] * 7,
        out_specs=any_spec,
        scratch_shapes=[
            pltpu.VMEM((B, D), dt),
            pltpu.VMEM((_NBUF, W, DH), dt),
            pltpu.VMEM((_NBUF, W, DH), dt),
            pltpu.VMEM((D, H * DH), dt),
            pltpu.VMEM((H * DH, D), dt),
            pltpu.VMEM((F, D), dt),
            pltpu.VMEM((F, D), dt),
            pltpu.VMEM((H, 8, DH), jnp.float32),
            pltpu.VMEM((H, 8, DH), jnp.float32),
            pltpu.VMEM((B, D), dt),
            pltpu.SemaphoreType.DMA((_NBUF,)),
            pltpu.SemaphoreType.DMA((_NBUF,)),
            pltpu.SemaphoreType.DMA((5,)),
            pltpu.SemaphoreType.DMA((_WO_CHUNKS,)),
        ],
        compiler_params=pltpu.CompilerParams(vmem_limit_bytes=64 * 1024 * 1024),
    )(A_x.reshape(B, D), A_k_cache, A_v_cache, A_wq, A_wo, B_w3.T, B_w4)
    return out.reshape(B, SQ, D)
```

```python
import jax
import jax.numpy as jnp
import jax.experimental.pallas as pl
import jax.experimental.pallas.tpu as pltpu

_EPS = 1e-5
_GH = 8
_ROWS = 16
_R = 256
_NB = 4
_WQ_SEG = 8
_W3_SEG = 2
_WO_ROWS = 32
_TAIL = (4, 3, 1)
_PROJ_STEP = 120


def _layernorm(x):
    m = jnp.mean(x, axis=-1, keepdims=True)
    xc = x - m
    v = jnp.mean(xc * xc, axis=-1, keepdims=True)
    return xc / jnp.sqrt(v + _EPS)


def _make_kernel(B, H, SK, DH, W, D, F):
    NG = B * H // _GH
    NR = W // _R
    NSTEP = NG * NR
    ND = _R // _ROWS
    AHEAD = _NB - 1
    EARLY_H = H - sum(_TAIL)
    N_WO_EARLY = EARLY_H * DH // _WO_ROWS
    N_W3 = F // _W3_SEG // 16
    WQ_COLS = 256
    N_WQ = (D // _WQ_SEG // 8) * (H * DH // WQ_COLS)
    WQ_CB = H * DH // WQ_COLS
    scale = DH ** -0.5
    bf16 = jnp.bfloat16
    f32 = jnp.float32
    assert N_WO_EARLY <= _PROJ_STEP < NSTEP and EARLY_H <= (_PROJ_STEP // (B * NR)) * _GH

    def kernel(x_hbm, k_hbm, v_hbm, wq_hbm, wo_hbm, w3_hbm, w4_hbm, out_hbm,
               x_buf, kbuf, vbuf, wq_buf, wo_buf, w3_buf, w4_buf,
               q_scr, o_scr, acc_scr, out_buf,
               sem_k, sem_v, sem_w, sem_wo):
        x_cp = pltpu.make_async_copy(x_hbm, x_buf, sem_w.at[0])
        out_cp = pltpu.make_async_copy(out_buf, out_hbm, sem_w.at[4])

        def kv_src(step):
            g = step // NR
            return (g % B) * H + (g // B) * _GH, SK - W + (step % NR) * _R

        def issue_kv(step, slot):
            p0, base = kv_src(step)

            def body(s, c):
                r0 = pl.multiple_of(s * _ROWS, _ROWS)
                src0 = pl.multiple_of(base + r0, _ROWS)
                pltpu.make_async_copy(k_hbm.at[pl.ds(p0, _GH), pl.ds(src0, _ROWS), :],
                                      kbuf.at[slot, :, pl.ds(r0, _ROWS), :],
                                      sem_k.at[slot]).start(priority=0)
                pltpu.make_async_copy(v_hbm.at[pl.ds(p0, _GH), pl.ds(src0, _ROWS), :],
                                      vbuf.at[slot, :, pl.ds(r0, _ROWS), :],
                                      sem_v.at[slot]).start(priority=1)
                return c
            jax.lax.fori_loop(0, ND, body, 0, unroll=4)

        def wo_desc(i, sem):
            r = pl.multiple_of(i * _WO_ROWS, _WO_ROWS)
            return pltpu.make_async_copy(wo_hbm.at[pl.ds(r, _WO_ROWS), :],
                                         wo_buf.at[pl.ds(r, _WO_ROWS), :], sem)

        def wq_desc(i):
            r = pl.multiple_of((i // WQ_CB) * 8, 8)
            c = pl.multiple_of((i % WQ_CB) * WQ_COLS, WQ_COLS)
            return pltpu.make_async_copy(wq_hbm.at[:, pl.ds(r, 8), pl.ds(c, WQ_COLS)],
                                         wq_buf.at[:, pl.ds(r, 8), pl.ds(c, WQ_COLS)], sem_w.at[3])

        def w_desc(src, dst, sem, i):
            r = pl.multiple_of(i * 16, 16)
            return pltpu.make_async_copy(src.at[:, pl.ds(r, 16), :], dst.at[:, pl.ds(r, 16), :], sem)

        def wait_filled(buf, sem):
            pltpu.make_async_copy(buf, buf, sem).wait()

        x_cp.start()

        def issue_wq(i, c):
            wq_desc(2 * i).start(priority=0)
            wq_desc(2 * i + 1).start(priority=1)
            return c
        jax.lax.fori_loop(0, N_WQ // 2, issue_wq, 0)

        def issue_w34(i, c):
            w_desc(w3_hbm, w3_buf, sem_w.at[1], i).start(priority=0)
            w_desc(w4_hbm, w4_buf, sem_w.at[2], i).start(priority=1)
            return c
        jax.lax.fori_loop(0, N_W3, issue_w34, 0)
        issue_kv(0, 0)

        x_cp.wait()
        x4 = x_buf[...].astype(f32)
        x8 = jnp.concatenate([x4, x4], axis=0)
        xn = _layernorm(x8)
        xn2 = _layernorm(xn)
        wait_filled(wq_buf, sem_w.at[3])
        q_all = jnp.dot(xn.astype(bf16), wq_buf[...].reshape(D, H * DH), preferred_element_type=f32)
        for h in range(H):
            q_scr[pl.ds(h, B, stride=H), :] = q_all[0:B, h * DH:(h + 1) * DH]
        for i in range(1, AHEAD):
            issue_kv(i, i)

        wait_filled(w3_buf, sem_w.at[1])
        hmid = jax.lax.dot_general(xn2.astype(bf16), w3_buf[...].reshape(F, D),
                                   (((1,), (1,)), ((), ())), preferred_element_type=f32)
        hmid = jax.nn.gelu(hmid, approximate=True)
        wait_filled(w4_buf, sem_w.at[2])
        mlp = jnp.dot(hmid.astype(bf16), w4_buf[...].reshape(F, D), preferred_element_type=f32)
        acc_scr[...] = (x8 + xn + mlp)[0:B]

        row = jax.lax.broadcasted_iota(jnp.int32, (_GH, DH), 0)

        def o_head(h):
            return o_scr[pl.ds(h, B, stride=H), :].astype(bf16)

        def project(h, oh, acc_out):
            return acc_out + jnp.dot(oh, wo_buf[h * DH:(h + 1) * DH, :], preferred_element_type=f32)

        def issue_tail_wo():
            i0 = N_WO_EARLY
            for t, nh in enumerate(_TAIL):
                n = nh * DH // _WO_ROWS
                for u in range(n):
                    wo_desc(i0 + u, sem_wo.at[1 + t]).start(priority=1)
                i0 += n

        def step_body(step, carry):
            m, l, acc = carry
            r = step % NR
            slot = step % _NB
            nxt = step + AHEAD

            @pl.when(nxt < NSTEP)
            def _():
                issue_kv(nxt, nxt % _NB)

            @pl.when(nxt == NSTEP)
            def _():
                issue_tail_wo()

            @pl.when(step < N_WO_EARLY)
            def _():
                wo_desc(step, sem_wo.at[0]).start(priority=0)

            p0, _ = kv_src(step)
            p0 = pl.multiple_of(p0, _GH)
            qg = q_scr[pl.ds(p0, _GH), :]
            wait_filled(kbuf.at[slot], sem_k.at[slot])
            s = None
            for j in range(_GH):
                lhs = jnp.where(row == j, qg, 0.0).astype(bf16)
                sj = jax.lax.dot_general(lhs, kbuf[slot, j], (((1,), (1,)), ((), ())),
                                         preferred_element_type=f32)
                s = sj if s is None else s + sj
            first = r == 0
            m_prev = jnp.where(first, -jnp.inf, m)
            m_new = jnp.maximum(m_prev, jnp.max(s, axis=-1, keepdims=True))
            p = jnp.exp((s - m_new) * scale)
            alpha = jnp.exp((m_prev - m_new) * scale)
            ps = p[:, 0:DH]
            for t in range(1, _R // DH):
                ps = ps + p[:, t * DH:(t + 1) * DH]
            pb = p.astype(bf16)
            wait_filled(vbuf.at[slot], sem_v.at[slot])
            o = None
            for j in range(_GH):
                oj = jnp.dot(pb, vbuf[slot, j], preferred_element_type=f32)
                o = oj if o is None else jnp.where(row == j, oj, o)
            l = jnp.where(first, ps, alpha * l + ps)
            acc = jnp.where(first, o, alpha * acc + o)

            @pl.when(r == NR - 1)
            def _():
                o_scr[pl.ds(p0, _GH), :] = acc / jnp.sum(l, axis=-1, keepdims=True)

            @pl.when(step == _PROJ_STEP)
            def _():
                wait_filled(wo_buf.at[pl.ds(0, EARLY_H * DH), :], sem_wo.at[0])
                a = acc_scr[...]
                for h in range(EARLY_H):
                    a = project(h, o_head(h), a)
                acc_scr[...] = a

            return m_new, l, acc

        init = (jnp.zeros((_GH, 1), f32), jnp.zeros((_GH, DH), f32), jnp.zeros((_GH, DH), f32))
        jax.lax.fori_loop(0, NSTEP, step_body, init)

        acc_out = acc_scr[...]
        ohs = [o_head(h) for h in range(EARLY_H, H)]
        h0 = EARLY_H
        for t, nh in enumerate(_TAIL):
            wait_filled(wo_buf.at[pl.ds(h0 * DH, nh * DH), :], sem_wo.at[1 + t])
            for h in range(h0, h0 + nh):
                acc_out = project(h, ohs[h - EARLY_H], acc_out)
            h0 += nh
        out_buf[...] = acc_out.astype(out_buf.dtype)
        out_cp.start()
        out_cp.wait()

    return kernel


@jax.jit
def pallas_parallel_sum__sliding_block_cached__mixer_s_mlp__decode_kernel(
    A_x: jax.Array,
    A_k_cache: jax.Array,
    A_v_cache: jax.Array,
    A_wq: jax.Array,
    A_wo: jax.Array,
    B_x: jax.Array,
    B_w1: jax.Array,
    B_w2: jax.Array,
    B_w3: jax.Array,
    B_w4: jax.Array,
):
    B, SQ, D = A_x.shape
    _, H, SK, DH = A_k_cache.shape
    F = B_w3.shape[1]
    W = min(4096, max(256, SK // 4))
    dt = A_x.dtype
    assert SQ == 1 and 2 * B == _GH

    any_spec = pl.BlockSpec(memory_space=pl.ANY)
    out = pl.pallas_call(
        _make_kernel(B, H, SK, DH, W, D, F),
        out_shape=jax.ShapeDtypeStruct((B, D), dt),
        in_specs=[any_spec] * 7,
        out_specs=any_spec,
        scratch_shapes=[
            pltpu.VMEM((B, D), dt),
            pltpu.VMEM((_NB, _GH, _R, DH), dt),
            pltpu.VMEM((_NB, _GH, _R, DH), dt),
            pltpu.VMEM((_WQ_SEG, D // _WQ_SEG, H * DH), dt),
            pltpu.VMEM((H * DH, D), dt),
            pltpu.VMEM((_W3_SEG, F // _W3_SEG, D), dt),
            pltpu.VMEM((_W3_SEG, F // _W3_SEG, D), dt),
            pltpu.VMEM((B * H, DH), jnp.float32),
            pltpu.VMEM((B * H, DH), jnp.float32),
            pltpu.VMEM((B, D), jnp.float32),
            pltpu.VMEM((B, D), dt),
            pltpu.SemaphoreType.DMA((_NB,)),
            pltpu.SemaphoreType.DMA((_NB,)),
            pltpu.SemaphoreType.DMA((5,)),
            pltpu.SemaphoreType.DMA((1 + len(_TAIL),)),
        ],
        compiler_params=pltpu.CompilerParams(vmem_limit_bytes=64 * 1024 * 1024,
                                             disable_bounds_checks=True,
                                             disable_semaphore_checks=True),
    )(A_x.reshape(B, D), A_k_cache.reshape(B * H, SK, DH), A_v_cache.reshape(B * H, SK, DH),
      A_wq.reshape(_WQ_SEG, D // _WQ_SEG, H * DH), A_wo,
      B_w3.T.reshape(_W3_SEG, F // _W3_SEG, D), B_w4.reshape(_W3_SEG, F // _W3_SEG, D))
    return out.reshape(B, SQ, D)
```

```python
import jax
import jax.numpy as jnp
import jax.experimental.pallas as pl
import jax.experimental.pallas.tpu as pltpu

_EPS = 1e-5
_GH = 8
_ROWS = 16
_R = 256
_NB = 4
_WQ_SEG = 2
_W3_SEG = 2
_WO_ROWS = 32
_TAIL = (4, 3, 1)
_PROJ_STEP = 120


def _layernorm(x):
    m = jnp.mean(x, axis=-1, keepdims=True)
    xc = x - m
    v = jnp.mean(xc * xc, axis=-1, keepdims=True)
    return xc / jnp.sqrt(v + _EPS)


def _make_kernel(B, H, SK, DH, W, D, F):
    NG = B * H // _GH
    NR = W // _R
    NSTEP = NG * NR
    ND = _R // _ROWS
    AHEAD = _NB - 1
    EARLY_H = H - sum(_TAIL)
    N_WO_EARLY = EARLY_H * DH // _WO_ROWS
    N_W3 = F // _W3_SEG // 16
    WQ_COLS = 1024
    N_WQ = (D // _WQ_SEG // 8) * (H * DH // WQ_COLS)
    WQ_CB = H * DH // WQ_COLS
    scale = DH ** -0.5
    bf16 = jnp.bfloat16
    f32 = jnp.float32
    assert N_WO_EARLY <= _PROJ_STEP < NSTEP and EARLY_H <= (_PROJ_STEP // (B * NR)) * _GH

    def kernel(x_hbm, k_hbm, v_hbm, wq_hbm, wo_hbm, w3_hbm, w4_hbm, out_hbm,
               x_buf, kbuf, vbuf, wq_buf, wo_buf, w3_buf, w4_buf,
               q_scr, o_scr, acc_scr, out_buf,
               sem_k, sem_v, sem_w, sem_wo):
        x_cp = pltpu.make_async_copy(x_hbm, x_buf, sem_w.at[0])
        out_cp = pltpu.make_async_copy(out_buf, out_hbm, sem_w.at[4])

        def kv_src(step):
            g = step // NR
            return (g % B) * H + (g // B) * _GH, SK - W + (step % NR) * _R

        def issue_kv(step, slot):
            p0, base = kv_src(step)

            def body(s, c):
                r0 = pl.multiple_of(s * _ROWS, _ROWS)
                src0 = pl.multiple_of(base + r0, _ROWS)
                pltpu.make_async_copy(k_hbm.at[pl.ds(p0, _GH), pl.ds(src0, _ROWS), :],
                                      kbuf.at[slot, :, pl.ds(r0, _ROWS), :],
                                      sem_k.at[slot]).start(priority=0)
                pltpu.make_async_copy(v_hbm.at[pl.ds(p0, _GH), pl.ds(src0, _ROWS), :],
                                      vbuf.at[slot, :, pl.ds(r0, _ROWS), :],
                                      sem_v.at[slot]).start(priority=1)
                return c
            jax.lax.fori_loop(0, ND, body, 0, unroll=4)

        def wo_desc(i, sem):
            r = pl.multiple_of(i * _WO_ROWS, _WO_ROWS)
            return pltpu.make_async_copy(wo_hbm.at[pl.ds(r, _WO_ROWS), :],
                                         wo_buf.at[pl.ds(r, _WO_ROWS), :], sem)

        def wq_desc(i):
            r = pl.multiple_of((i // WQ_CB) * 8, 8)
            c = pl.multiple_of((i % WQ_CB) * WQ_COLS, WQ_COLS)
            return pltpu.make_async_copy(wq_hbm.at[:, pl.ds(r, 8), pl.ds(c, WQ_COLS)],
                                         wq_buf.at[:, pl.ds(r, 8), pl.ds(c, WQ_COLS)], sem_w.at[3])

        def w_desc(src, dst, sem, i):
            r = pl.multiple_of(i * 16, 16)
            return pltpu.make_async_copy(src.at[:, pl.ds(r, 16), :], dst.at[:, pl.ds(r, 16), :], sem)

        def wait_filled(buf, sem):
            pltpu.make_async_copy(buf, buf, sem).wait()

        x_cp.start()

        def issue_wq(i, c):
            wq_desc(i).start(priority=0)
            wq_desc(N_WQ // 2 + i).start(priority=1)
            return c
        jax.lax.fori_loop(0, N_WQ // 2, issue_wq, 0)

        def issue_w34(i, c):
            w_desc(w3_hbm, w3_buf, sem_w.at[1], i).start(priority=0)
            w_desc(w4_hbm, w4_buf, sem_w.at[2], i).start(priority=1)
            return c
        jax.lax.fori_loop(0, N_W3, issue_w34, 0)
        issue_kv(0, 0)

        x_cp.wait()
        x4 = x_buf[...].astype(f32)
        x8 = jnp.concatenate([x4, x4], axis=0)
        xn = _layernorm(x8)
        xn2 = _layernorm(xn)
        wait_filled(wq_buf, sem_w.at[3])
        q_all = jnp.dot(xn.astype(bf16), wq_buf[...].reshape(D, H * DH), preferred_element_type=f32)
        for h in range(H):
            q_scr[pl.ds(h, B, stride=H), :] = q_all[0:B, h * DH:(h + 1) * DH]
        for i in range(1, AHEAD):
            issue_kv(i, i)

        wait_filled(w3_buf, sem_w.at[1])
        hmid = jax.lax.dot_general(xn2.astype(bf16), w3_buf[...].reshape(F, D),
                                   (((1,), (1,)), ((), ())), preferred_element_type=f32)
        hmid = jax.nn.gelu(hmid, approximate=True)
        wait_filled(w4_buf, sem_w.at[2])
        mlp = jnp.dot(hmid.astype(bf16), w4_buf[...].reshape(F, D), preferred_element_type=f32)
        acc_scr[...] = (x8 + xn + mlp)[0:B]

        row = jax.lax.broadcasted_iota(jnp.int32, (_GH, DH), 0)

        def o_head(h):
            return o_scr[pl.ds(h, B, stride=H), :].astype(bf16)

        def project(h, oh, acc_out):
            return acc_out + jnp.dot(oh, wo_buf[h * DH:(h + 1) * DH, :], preferred_element_type=f32)

        def issue_tail_wo():
            i0 = N_WO_EARLY
            for t, nh in enumerate(_TAIL):
                n = nh * DH // _WO_ROWS
                for u in range(n):
                    wo_desc(i0 + u, sem_wo.at[1 + t]).start(priority=1)
                i0 += n

        def step_body(step, carry):
            m, l, acc = carry
            r = step % NR
            slot = step % _NB
            nxt = step + AHEAD

            @pl.when(nxt < NSTEP)
            def _():
                issue_kv(nxt, nxt % _NB)

            @pl.when(nxt == NSTEP)
            def _():
                issue_tail_wo()

            @pl.when(step < N_WO_EARLY)
            def _():
                wo_desc(step, sem_wo.at[0]).start(priority=0)

            p0, _ = kv_src(step)
            p0 = pl.multiple_of(p0, _GH)
            qg = q_scr[pl.ds(p0, _GH), :]
            wait_filled(kbuf.at[slot], sem_k.at[slot])
            s = None
            for j in range(_GH):
                lhs = jnp.where(row == j, qg, 0.0).astype(bf16)
                sj = jax.lax.dot_general(lhs, kbuf[slot, j], (((1,), (1,)), ((), ())),
                                         preferred_element_type=f32)
                s = sj if s is None else s + sj
            first = r == 0
            m_prev = jnp.where(first, -jnp.inf, m)
            m_new = jnp.maximum(m_prev, jnp.max(s, axis=-1, keepdims=True))
            p = jnp.exp((s - m_new) * scale)
            alpha = jnp.exp((m_prev - m_new) * scale)
            ps = p[:, 0:DH]
            for t in range(1, _R // DH):
                ps = ps + p[:, t * DH:(t + 1) * DH]
            pb = p.astype(bf16)
            wait_filled(vbuf.at[slot], sem_v.at[slot])
            o = None
            for j in range(_GH):
                oj = jnp.dot(pb, vbuf[slot, j], preferred_element_type=f32)
                o = oj if o is None else jnp.where(row == j, oj, o)
            l = jnp.where(first, ps, alpha * l + ps)
            acc = jnp.where(first, o, alpha * acc + o)

            @pl.when(r == NR - 1)
            def _():
                o_scr[pl.ds(p0, _GH), :] = acc / jnp.sum(l, axis=-1, keepdims=True)

            @pl.when(step == _PROJ_STEP)
            def _():
                wait_filled(wo_buf.at[pl.ds(0, EARLY_H * DH), :], sem_wo.at[0])
                a = acc_scr[...]
                for h in range(EARLY_H):
                    a = project(h, o_head(h), a)
                acc_scr[...] = a

            return m_new, l, acc

        init = (jnp.zeros((_GH, 1), f32), jnp.zeros((_GH, DH), f32), jnp.zeros((_GH, DH), f32))
        jax.lax.fori_loop(0, NSTEP, step_body, init)

        acc_out = acc_scr[...]
        ohs = [o_head(h) for h in range(EARLY_H, H)]
        h0 = EARLY_H
        for t, nh in enumerate(_TAIL):
            wait_filled(wo_buf.at[pl.ds(h0 * DH, nh * DH), :], sem_wo.at[1 + t])
            for h in range(h0, h0 + nh):
                acc_out = project(h, ohs[h - EARLY_H], acc_out)
            h0 += nh
        out_buf[...] = acc_out.astype(out_buf.dtype)
        out_cp.start()
        out_cp.wait()

    return kernel


@jax.jit
def pallas_parallel_sum__sliding_block_cached__mixer_s_mlp__decode_kernel(
    A_x: jax.Array,
    A_k_cache: jax.Array,
    A_v_cache: jax.Array,
    A_wq: jax.Array,
    A_wo: jax.Array,
    B_x: jax.Array,
    B_w1: jax.Array,
    B_w2: jax.Array,
    B_w3: jax.Array,
    B_w4: jax.Array,
):
    B, SQ, D = A_x.shape
    _, H, SK, DH = A_k_cache.shape
    F = B_w3.shape[1]
    W = min(4096, max(256, SK // 4))
    dt = A_x.dtype
    assert SQ == 1 and 2 * B == _GH

    any_spec = pl.BlockSpec(memory_space=pl.ANY)
    out = pl.pallas_call(
        _make_kernel(B, H, SK, DH, W, D, F),
        out_shape=jax.ShapeDtypeStruct((B, D), dt),
        in_specs=[any_spec] * 7,
        out_specs=any_spec,
        scratch_shapes=[
            pltpu.VMEM((B, D), dt),
            pltpu.VMEM((_NB, _GH, _R, DH), dt),
            pltpu.VMEM((_NB, _GH, _R, DH), dt),
            pltpu.VMEM((_WQ_SEG, D // _WQ_SEG, H * DH), dt),
            pltpu.VMEM((H * DH, D), dt),
            pltpu.VMEM((_W3_SEG, F // _W3_SEG, D), dt),
            pltpu.VMEM((_W3_SEG, F // _W3_SEG, D), dt),
            pltpu.VMEM((B * H, DH), jnp.float32),
            pltpu.VMEM((B * H, DH), jnp.float32),
            pltpu.VMEM((B, D), jnp.float32),
            pltpu.VMEM((B, D), dt),
            pltpu.SemaphoreType.DMA((_NB,)),
            pltpu.SemaphoreType.DMA((_NB,)),
            pltpu.SemaphoreType.DMA((5,)),
            pltpu.SemaphoreType.DMA((1 + len(_TAIL),)),
        ],
        compiler_params=pltpu.CompilerParams(vmem_limit_bytes=64 * 1024 * 1024,
                                             disable_bounds_checks=True,
                                             disable_semaphore_checks=True),
    )(A_x.reshape(B, D), A_k_cache.reshape(B * H, SK, DH), A_v_cache.reshape(B * H, SK, DH),
      A_wq.reshape(_WQ_SEG, D // _WQ_SEG, H * DH), A_wo,
      B_w3.T.reshape(_W3_SEG, F // _W3_SEG, D), B_w4.reshape(_W3_SEG, F // _W3_SEG, D))
    return out.reshape(B, SQ, D)
```
